```python
import os as _os
_os.environ.setdefault("JAX_PLATFORMS", "cpu")
import jax
import jax.numpy as jnp

def _softmax(x, axis=-1):
    return jax.nn.softmax(x, axis=axis)
def _gelu(x):
    return jax.nn.gelu(x, approximate=True)
def _silu(x):
    return jax.nn.silu(x)
def _sigmoid(x):
    return jax.nn.sigmoid(x)
def _layernorm(x, axis=-1, eps=1e-5):
    m = jnp.mean(x, axis=axis, keepdims=True)
    v = jnp.var(x, axis=axis, keepdims=True)
    return (x - m) / jnp.sqrt(v + eps)
def _scatter_add(tgt, idx, src, axis=0):
    return tgt.at[idx].add(src)
def _segment_sum(src, seg, n):
    return jax.ops.segment_sum(src, seg, n)
class _Rng:
    def __init__(self, key):
        self._k = key
    def _next(self):
        self._k, sub = jax.random.split(self._k)
        return sub
    def normal(self, shape):
        return jax.random.normal(self._next(), shape, dtype=jnp.bfloat16)
    def randint(self, lo, hi, shape):
        return jax.random.randint(self._next(), shape, lo, hi, dtype=jnp.int32)
    def uniform(self, shape, lo=0.0, hi=1.0):
        return jax.random.uniform(self._next(), shape, jnp.bfloat16, lo, hi)
    def permutation(self, n):
        return jax.random.permutation(self._next(), n)


kernel_name = 'concat_heads__sliding_block_cached__sliding_block_cached__decode'

def setup_inputs():
    _rng = _Rng(jax.random.key(int.from_bytes(__import__("os").urandom(4), "little")))
    _w = (lambda a: (lambda t: t.astype(jnp.bfloat16) if jnp.issubdtype(t.dtype, jnp.floating) else t)(jnp.asarray(a)))
    def _A_setup():
        B, Sq, D = 2, 1, 640
        Hq, Hkv, Sk, Dh = 32, 32, 4096, 128
        assert Hq % Hkv == 0, (Hq, Hkv)
        return {
            "x": _w((lambda *s: _rng.normal(s) * 0.8)(B, Sq, D)),
            "k_cache": _w((lambda *s: _rng.normal(s) * 0.8)(B, Hkv, Sk, Dh)),
            "v_cache": _w((lambda *s: _rng.normal(s) * 0.05)(B, Hkv, Sk, Dh)),
            "wq": _w((lambda *s: _rng.normal(s) * 0.8)(D, Hq * Dh) * (D ** -0.5)),
            "wo": _w((lambda *s: _rng.normal(s) * 0.05)(Hq * Dh, D) * ((Hq * Dh) ** -0.5)),
        }
    _A_in = _A_setup()

    def _B_setup():
        B, Sq, D = 2, 1, 640
        Hq, Hkv, Sk, Dh = 32, 32, 4096, 128
        assert Hq % Hkv == 0, (Hq, Hkv)
        return {
            "x": _w((lambda *s: _rng.normal(s) * 0.8)(B, Sq, D)),
            "k_cache": _w((lambda *s: _rng.normal(s) * 0.8)(B, Hkv, Sk, Dh)),
            "v_cache": _w((lambda *s: _rng.normal(s) * 0.05)(B, Hkv, Sk, Dh)),
            "wq": _w((lambda *s: _rng.normal(s) * 0.8)(D, Hq * Dh) * (D ** -0.5)),
            "wo": _w((lambda *s: _rng.normal(s) * 0.05)(Hq * Dh, D) * ((Hq * Dh) ** -0.5)),
        }
    _B_in = _B_setup()

    return {
        "A_x": _A_in["x"],
        "A_k_cache": _A_in["k_cache"],
        "A_v_cache": _A_in["v_cache"],
        "A_wq": _A_in["wq"],
        "A_wo": _A_in["wo"],
        "B_x": _B_in["x"],
        "B_k_cache": _B_in["k_cache"],
        "B_v_cache": _B_in["v_cache"],
        "B_wq": _B_in["wq"],
        "B_wo": _B_in["wo"],
    }

def reference(A_x, A_k_cache, A_v_cache, A_wq, A_wo, B_x, B_k_cache, B_v_cache, B_wq, B_wo):
    def _A_ref(x, k_cache, v_cache, wq, wo):
        B, Sq, D = x.shape
        Hq, Dh = 32, 128
        Hkv, Sk = k_cache.shape[1], k_cache.shape[2]
        W = min(4096, max(256, Sk // 4))
        rep = Hq // Hkv
        q = (lambda x, *d: x.transpose(*d))((x @ wq).reshape(B, Sq, Hq, Dh), 0, 2, 1, 3)
        k = jnp.repeat(k_cache[:, :, Sk - W:, :], rep, axis=1)
        v = jnp.repeat(v_cache[:, :, Sk - W:, :], rep, axis=1)
        scores = jnp.einsum("bhqd,bhkd->bhqk", q, k) * (Dh ** -0.5)
        p = _softmax(scores, axis=-1)
        o = jnp.einsum("bhqk,bhkd->bhqd", p, v)
        return (lambda x, *d: x.transpose(*d))(o, 0, 2, 1, 3).reshape(B, Sq, Hq * Dh) @ wo

    def _B_ref(x, k_cache, v_cache, wq, wo):
        B, Sq, D = x.shape
        Hq, Dh = 32, 128
        Hkv, Sk = k_cache.shape[1], k_cache.shape[2]
        W = min(4096, max(256, Sk // 4))
        rep = Hq // Hkv
        q = (lambda x, *d: x.transpose(*d))((x @ wq).reshape(B, Sq, Hq, Dh), 0, 2, 1, 3)
        k = jnp.repeat(k_cache[:, :, Sk - W:, :], rep, axis=1)
        v = jnp.repeat(v_cache[:, :, Sk - W:, :], rep, axis=1)
        scores = jnp.einsum("bhqd,bhkd->bhqk", q, k) * (Dh ** -0.5)
        p = _softmax(scores, axis=-1)
        o = jnp.einsum("bhqk,bhkd->bhqd", p, v)
        return (lambda x, *d: x.transpose(*d))(o, 0, 2, 1, 3).reshape(B, Sq, Hq * Dh) @ wo

    a = _A_ref(A_x, A_k_cache, A_v_cache, A_wq, A_wo)
    b = _B_ref(B_x, B_k_cache, B_v_cache, B_wq, B_wo)
    return jnp.concatenate([a, b], axis=-1)
```

```python
import jax
import jax.numpy as jnp
from jax import lax
import jax.experimental.pallas as pl
import jax.experimental.pallas.tpu as pltpu


_HEADS_PER_DMA = 4


def _wo_chunks(rows, last):
    if not last:
        return (512,) * (rows // 512)
    return (512,) * (rows // 512 - 1) + (256, 128, 128)


@jax.jit
def pallas_concat_heads__sliding_block_cached__sliding_block_cached__decode_kernel(
    A_x: jax.Array,
    A_k_cache: jax.Array,
    A_v_cache: jax.Array,
    A_wq: jax.Array,
    A_wo: jax.Array,
    B_x: jax.Array,
    B_k_cache: jax.Array,
    B_v_cache: jax.Array,
    B_wq: jax.Array,
    B_wo: jax.Array,
):
    B, Sq, D = A_x.shape
    _, H, Sk, Dh = A_k_cache.shape
    assert Sq == 1 and H == 32 and Dh == 128
    W = min(4096, max(256, Sk // 4))
    HD = H * Dh
    scale = Dh ** -0.5
    G = _HEADS_PER_DMA
    NG = H // G
    wo_chunks = (_wo_chunks(HD, False), _wo_chunks(HD, True))
    wo_offs = tuple(
        tuple(sum(ch[:c]) for c in range(len(ch))) for ch in wo_chunks
    )
    n_wo = max(len(ch) for ch in wo_chunks)
    cdtype = A_x.dtype

    def kernel_function(ax, ak, av, awq, awo, bx, bk, bv, bwq, bwo, o_ref,
                        xbuf, kvbuf, wqbuf, wobuf, obuf):
        xs = (ax, bx)
        kvs = (ak, av, bk, bv)
        wqs = (awq, bwq)
        wos = (awo, bwo)

        def inner(xsem, wqsem, kvsem, wosem):
            def x_copy(p):
                return pltpu.make_async_copy(xs[p], xbuf.at[p], xsem.at[p])

            def wq_copy(p):
                return pltpu.make_async_copy(wqs[p], wqbuf.at[p], wqsem.at[p])

            def kv_copy(t, g):
                return pltpu.make_async_copy(
                    kvs[t].at[:, pl.ds(g * G, G), pl.ds(Sk - W, W), :],
                    kvbuf.at[t, :, pl.ds(g * G, G)],
                    kvsem.at[t, g],
                )

            def wo_copy(p, c):
                rows = pl.ds(wo_offs[p][c], wo_chunks[p][c])
                return pltpu.make_async_copy(
                    wos[p].at[rows], wobuf.at[p, rows], wosem.at[p, c]
                )

            for p in range(2):
                x_copy(p).start()
            for p in range(2):
                wq_copy(p).start()
            for g in range(NG):
                for t in range(4):
                    kv_copy(t, g).start()
            for p in range(2):
                for c in range(len(wo_chunks[p])):
                    wo_copy(p, c).start()

            for p in range(2):
                x_copy(p).wait()
            for p in range(2):
                wq_copy(p).wait()

            def group_body(g, carry):
                for p in range(2):
                    kv_copy(2 * p, g).wait()
                    kv_copy(2 * p + 1, g).wait()
                    for j in range(G):
                        h = g * G + j
                        col = pl.multiple_of(h * Dh, Dh)
                        q = jnp.dot(
                            xbuf[p], wqbuf[p, :, pl.ds(col, Dh)],
                            preferred_element_type=jnp.float32,
                        ).astype(cdtype)
                        rows = []
                        for b in range(B):
                            s = lax.dot_general(
                                q[b:b + 1, :], kvbuf[2 * p, b, h],
                                (((1,), (1,)), ((), ())),
                                preferred_element_type=jnp.float32,
                            ) * scale
                            m = jnp.max(s, axis=-1, keepdims=True)
                            e = jnp.exp(s - m)
                            l = jnp.sum(e, axis=-1, keepdims=True)
                            o = jnp.dot(
                                e.astype(cdtype), kvbuf[2 * p + 1, b, h],
                                preferred_element_type=jnp.float32,
                            ) / l
                            rows.append(o)
                        obuf[p, :, pl.ds(col, Dh)] = jnp.concatenate(
                            rows, axis=0).astype(cdtype)
                return carry

            lax.fori_loop(0, NG, group_body, 0)

            for p in range(2):
                acc = jnp.zeros((B, D), jnp.float32)
                for c in range(len(wo_chunks[p])):
                    rows = pl.ds(wo_offs[p][c], wo_chunks[p][c])
                    wo_copy(p, c).wait()
                    acc = acc + jnp.dot(
                        obuf[p, :, rows], wobuf[p, rows, :],
                        preferred_element_type=jnp.float32,
                    )
                o_ref[:, p * D:(p + 1) * D] = acc.astype(o_ref.dtype)

        pl.run_scoped(
            inner,
            pltpu.SemaphoreType.DMA((2,)),
            pltpu.SemaphoreType.DMA((2,)),
            pltpu.SemaphoreType.DMA((4, NG)),
            pltpu.SemaphoreType.DMA((2, n_wo)),
        )

    any_spec = pl.BlockSpec(memory_space=pl.ANY)
    out = pl.pallas_call(
        kernel_function,
        in_specs=[any_spec] * 10,
        out_specs=pl.BlockSpec((B, 2 * D), lambda: (0, 0)),
        out_shape=jax.ShapeDtypeStruct((B, 2 * D), cdtype),
        scratch_shapes=[
            pltpu.VMEM((2, B, D), cdtype),
            pltpu.VMEM((4, B, H, W, Dh), cdtype),
            pltpu.VMEM((2, D, HD), cdtype),
            pltpu.VMEM((2, HD, D), cdtype),
            pltpu.VMEM((2, B, HD), cdtype),
        ],
        compiler_params=pltpu.CompilerParams(
            vmem_limit_bytes=110 * 1024 * 1024),
    )(A_x.reshape(B, D), A_k_cache, A_v_cache, A_wq, A_wo,
      B_x.reshape(B, D), B_k_cache, B_v_cache, B_wq, B_wo)
    return out.reshape(B, 1, 2 * D)
```

```python
import jax
import jax.numpy as jnp
from jax import lax
import jax.experimental.pallas as pl
import jax.experimental.pallas.tpu as pltpu


_HEADS_PER_DMA = 4
_WO_CHUNK = 512
_WO_MXU_TAIL = (256, 128)
_WO_VPU_TAIL = (64, 32, 32)


@jax.jit
def pallas_concat_heads__sliding_block_cached__sliding_block_cached__decode_kernel(
    A_x: jax.Array,
    A_k_cache: jax.Array,
    A_v_cache: jax.Array,
    A_wq: jax.Array,
    A_wo: jax.Array,
    B_x: jax.Array,
    B_k_cache: jax.Array,
    B_v_cache: jax.Array,
    B_wq: jax.Array,
    B_wo: jax.Array,
):
    B, Sq, D = A_x.shape
    _, H, Sk, Dh = A_k_cache.shape
    assert Sq == 1 and H == 32 and Dh == 128 and D % 128 == 0
    W = min(4096, max(256, Sk // 4))
    HD = H * Dh
    scale = Dh ** -0.5
    G = _HEADS_PER_DMA
    NG = H // G
    RV = sum(_WO_VPU_TAIL)
    assert RV == 128
    n_full = (HD - sum(_WO_MXU_TAIL) - RV) // _WO_CHUNK
    wo_chunks = (
        (_WO_CHUNK,) * (HD // _WO_CHUNK),
        (_WO_CHUNK,) * n_full + _WO_MXU_TAIL + _WO_VPU_TAIL,
    )
    assert all(sum(ch) == HD for ch in wo_chunks)
    wo_offs = tuple(
        tuple(sum(ch[:c]) for c in range(len(ch))) for ch in wo_chunks
    )
    n_wo0 = len(wo_chunks[0])
    n_wo = n_wo0 + len(wo_chunks[1])
    n_mxu = (n_wo0, len(wo_chunks[1]) - len(_WO_VPU_TAIL))
    cdtype = A_x.dtype
    f32 = jnp.float32

    def kernel_function(ax, ak, av, awq, awo, bx, bk, bv, bwq, bwo, o_ref,
                        xbuf, kvbuf, wqbuf, wobuf, obuf):
        xs = (ax, bx)
        kvs = (ak, av, bk, bv)
        wqs = (awq, bwq)
        wos = (awo, bwo)

        def inner(hsem, kvsem, wosem):
            def x_copy(p):
                return pltpu.make_async_copy(xs[p], xbuf.at[p], hsem.at[p])

            def wq_copy(p):
                return pltpu.make_async_copy(wqs[p], wqbuf.at[p], hsem.at[2 + p])

            def kv_copy(t, g):
                heads = pl.ds(g * G, G)
                return pltpu.make_async_copy(
                    kvs[t].at[:, heads, pl.ds(Sk - W, W), :],
                    kvbuf.at[t, :, heads],
                    kvsem.at[g * 4 + t],
                )

            def wo_copy(p, c):
                rows = pl.ds(wo_offs[p][c], wo_chunks[p][c])
                return pltpu.make_async_copy(
                    wos[p].at[rows], wobuf.at[p, rows], wosem.at[p * n_wo0 + c]
                )

            for p in range(2):
                x_copy(p).start()
            for p in range(2):
                wq_copy(p).start()

            def issue_body(g, carry):
                for t in range(4):
                    kv_copy(t, g).start()
                return carry

            lax.fori_loop(0, NG, issue_body, 0)
            for p in range(2):
                for c in range(len(wo_chunks[p])):
                    wo_copy(p, c).start()

            for p in range(2):
                x_copy(p).wait()
            for p in range(2):
                wq_copy(p).wait()

            def group_body(g, carry):
                for p in range(2):
                    kv_copy(2 * p, g).wait()
                    kv_copy(2 * p + 1, g).wait()
                    for j in range(G):
                        h = g * G + j
                        col = pl.multiple_of(h * Dh, Dh)
                        q = jnp.dot(
                            xbuf[p], wqbuf[p, :, pl.ds(col, Dh)],
                            preferred_element_type=f32,
                        ).astype(cdtype)
                        rows = []
                        for b in range(B):
                            s = lax.dot_general(
                                q[b:b + 1, :], kvbuf[2 * p, b, h],
                                (((1,), (1,)), ((), ())),
                                preferred_element_type=f32,
                            ) * scale
                            m = jnp.max(s, axis=-1, keepdims=True)
                            e = jnp.exp(s - m)
                            l = jnp.sum(e, axis=-1, keepdims=True)
                            o = jnp.dot(
                                e.astype(cdtype), kvbuf[2 * p + 1, b, h],
                                preferred_element_type=f32,
                            ) / l
                            rows.append(o)
                        obuf[p, :, pl.ds(col, Dh)] = jnp.concatenate(
                            rows, axis=0).astype(cdtype)
                return carry

            lax.fori_loop(0, NG, group_body, 0)

            olast = obuf[1, :, pl.ds(HD - RV, RV)].astype(f32)
            ocols = [
                jnp.broadcast_to(olast[b:b + 1, :], (RV, RV)).T
                for b in range(B)
            ]

            for p in range(2):
                acc = jnp.zeros((B, D), f32)
                for c in range(n_mxu[p]):
                    rows = pl.ds(wo_offs[p][c], wo_chunks[p][c])
                    wo_copy(p, c).wait()
                    acc = acc + jnp.dot(
                        obuf[p, :, rows], wobuf[p, rows, :],
                        preferred_element_type=f32,
                    )
                if n_mxu[p] < len(wo_chunks[p]):
                    acc8 = [jnp.zeros((8, D), f32) for _ in range(B)]
                    for c in range(n_mxu[p], len(wo_chunks[p])):
                        off, n = wo_offs[p][c], wo_chunks[p][c]
                        r0 = off - (HD - RV)
                        wo_copy(p, c).wait()
                        w = wobuf[p, pl.ds(off, n), :].astype(f32)
                        for b in range(B):
                            oc = jnp.concatenate(
                                [ocols[b][r0:r0 + n, :]] * (D // 128), axis=1)
                            acc8[b] = acc8[b] + (w * oc).reshape(
                                n // 8, 8, D).sum(axis=0)
                    acc = acc + jnp.concatenate(
                        [jnp.sum(a, axis=0, keepdims=True) for a in acc8],
                        axis=0)
                o_ref[:, p * D:(p + 1) * D] = acc.astype(o_ref.dtype)

        pl.run_scoped(
            inner,
            pltpu.SemaphoreType.DMA((4,)),
            pltpu.SemaphoreType.DMA((4 * NG,)),
            pltpu.SemaphoreType.DMA((n_wo,)),
        )

    any_spec = pl.BlockSpec(memory_space=pl.ANY)
    out = pl.pallas_call(
        kernel_function,
        in_specs=[any_spec] * 10,
        out_specs=pl.BlockSpec((B, 2 * D), lambda: (0, 0)),
        out_shape=jax.ShapeDtypeStruct((B, 2 * D), cdtype),
        scratch_shapes=[
            pltpu.VMEM((2, B, D), cdtype),
            pltpu.VMEM((4, B, H, W, Dh), cdtype),
            pltpu.VMEM((2, D, HD), cdtype),
            pltpu.VMEM((2, HD, D), cdtype),
            pltpu.VMEM((2, B, HD), cdtype),
        ],
        compiler_params=pltpu.CompilerParams(
            vmem_limit_bytes=110 * 1024 * 1024),
    )(A_x.reshape(B, D), A_k_cache, A_v_cache, A_wq, A_wo,
      B_x.reshape(B, D), B_k_cache, B_v_cache, B_wq, B_wo)
    return out.reshape(B, 1, 2 * D)
```

```python
import jax
import jax.numpy as jnp
import numpy as np
from jax import lax
import jax.experimental.pallas as pl
import jax.experimental.pallas.tpu as pltpu


_HEADS_PER_DMA = 4
_WO_CHUNK = 512
_WO_MXU_TAIL = (256, 128)
_WO_VPU_TAIL = (64, 32, 32)


@jax.jit
def pallas_concat_heads__sliding_block_cached__sliding_block_cached__decode_kernel(
    A_x: jax.Array,
    A_k_cache: jax.Array,
    A_v_cache: jax.Array,
    A_wq: jax.Array,
    A_wo: jax.Array,
    B_x: jax.Array,
    B_k_cache: jax.Array,
    B_v_cache: jax.Array,
    B_wq: jax.Array,
    B_wo: jax.Array,
):
    B, Sq, D = A_x.shape
    _, H, Sk, Dh = A_k_cache.shape
    assert Sq == 1 and H == 32 and Dh == 128 and D % 128 == 0
    W = min(4096, max(256, Sk // 4))
    HD = H * Dh
    G = _HEADS_PER_DMA
    NG = H // G
    RV = sum(_WO_VPU_TAIL)
    assert RV == 128
    n_full = (HD - sum(_WO_MXU_TAIL) - RV) // _WO_CHUNK
    wo_chunks = (
        (_WO_CHUNK,) * (HD // _WO_CHUNK),
        (_WO_CHUNK,) * n_full + _WO_MXU_TAIL + _WO_VPU_TAIL,
    )
    assert all(sum(ch) == HD for ch in wo_chunks)
    wo_offs = tuple(
        tuple(sum(ch[:c]) for c in range(len(ch))) for ch in wo_chunks
    )
    n_wo0 = len(wo_chunks[0])
    n_wo = n_wo0 + len(wo_chunks[1])
    n_mxu = (n_wo0, len(wo_chunks[1]) - len(_WO_VPU_TAIL))
    cdtype = A_x.dtype
    f32 = jnp.float32
    scale = float(np.asarray(Dh ** -0.5, dtype=cdtype))

    def rnd(v):
        return v.astype(cdtype).astype(f32)

    def kernel_function(ax, ak, av, awq, awo, bx, bk, bv, bwq, bwo, o_ref,
                        xbuf, kvbuf, wqbuf, wobuf, obuf):
        xs = (ax, bx)
        kvs = (ak, av, bk, bv)
        wqs = (awq, bwq)
        wos = (awo, bwo)

        def inner(hsem, kvsem, wosem):
            def x_copy(p):
                return pltpu.make_async_copy(xs[p], xbuf.at[p], hsem.at[p])

            def wq_copy(p):
                return pltpu.make_async_copy(wqs[p], wqbuf.at[p], hsem.at[2 + p])

            def kv_copy(t, g):
                heads = pl.ds(g * G, G)
                return pltpu.make_async_copy(
                    kvs[t].at[:, heads, pl.ds(Sk - W, W), :],
                    kvbuf.at[t, :, heads],
                    kvsem.at[g * 4 + t],
                )

            def wo_copy(p, c):
                rows = pl.ds(wo_offs[p][c], wo_chunks[p][c])
                return pltpu.make_async_copy(
                    wos[p].at[rows], wobuf.at[p, rows], wosem.at[p * n_wo0 + c]
                )

            for p in range(2):
                x_copy(p).start()
            for p in range(2):
                wq_copy(p).start()

            def issue_body(g, carry):
                for t in range(4):
                    kv_copy(t, g).start()
                return carry

            lax.fori_loop(0, NG, issue_body, 0)
            for p in range(2):
                for c in range(len(wo_chunks[p])):
                    wo_copy(p, c).start()

            for p in range(2):
                x_copy(p).wait()
            for p in range(2):
                wq_copy(p).wait()

            def group_body(g, carry):
                for p in range(2):
                    kv_copy(2 * p, g).wait()
                    kv_copy(2 * p + 1, g).wait()
                    for j in range(G):
                        h = g * G + j
                        col = pl.multiple_of(h * Dh, Dh)
                        q = jnp.dot(
                            xbuf[p], wqbuf[p, :, pl.ds(col, Dh)],
                            preferred_element_type=f32,
                        ).astype(cdtype)
                        rows = []
                        for b in range(B):
                            s = rnd(lax.dot_general(
                                q[b:b + 1, :], kvbuf[2 * p, b, h],
                                (((1,), (1,)), ((), ())),
                                preferred_element_type=f32,
                            ))
                            s = rnd(s * scale)
                            m = jnp.max(s, axis=-1, keepdims=True)
                            e = rnd(jnp.exp(rnd(s - m)))
                            l = rnd(jnp.sum(e, axis=-1, keepdims=True))
                            o = jnp.dot(
                                (e / l).astype(cdtype), kvbuf[2 * p + 1, b, h],
                                preferred_element_type=f32,
                            )
                            rows.append(o)
                        obuf[p, :, pl.ds(col, Dh)] = jnp.concatenate(
                            rows, axis=0).astype(cdtype)
                return carry

            lax.fori_loop(0, NG, group_body, 0)

            olast = obuf[1, :, pl.ds(HD - RV, RV)].astype(f32)
            ocols = [
                jnp.broadcast_to(olast[b:b + 1, :], (RV, RV)).T
                for b in range(B)
            ]

            for p in range(2):
                acc = jnp.zeros((B, D), f32)
                for c in range(n_mxu[p]):
                    rows = pl.ds(wo_offs[p][c], wo_chunks[p][c])
                    wo_copy(p, c).wait()
                    acc = acc + jnp.dot(
                        obuf[p, :, rows], wobuf[p, rows, :],
                        preferred_element_type=f32,
                    )
                if n_mxu[p] < len(wo_chunks[p]):
                    acc8 = [jnp.zeros((8, D), f32) for _ in range(B)]
                    for c in range(n_mxu[p], len(wo_chunks[p])):
                        off, n = wo_offs[p][c], wo_chunks[p][c]
                        r0 = off - (HD - RV)
                        wo_copy(p, c).wait()
                        w = wobuf[p, pl.ds(off, n), :].astype(f32)
                        for b in range(B):
                            oc = jnp.concatenate(
                                [ocols[b][r0:r0 + n, :]] * (D // 128), axis=1)
                            acc8[b] = acc8[b] + (w * oc).reshape(
                                n // 8, 8, D).sum(axis=0)
                    acc = acc + jnp.concatenate(
                        [jnp.sum(a, axis=0, keepdims=True) for a in acc8],
                        axis=0)
                o_ref[:, p * D:(p + 1) * D] = acc.astype(o_ref.dtype)

        pl.run_scoped(
            inner,
            pltpu.SemaphoreType.DMA((4,)),
            pltpu.SemaphoreType.DMA((4 * NG,)),
            pltpu.SemaphoreType.DMA((n_wo,)),
        )

    any_spec = pl.BlockSpec(memory_space=pl.ANY)
    out = pl.pallas_call(
        kernel_function,
        in_specs=[any_spec] * 10,
        out_specs=pl.BlockSpec((B, 2 * D), lambda: (0, 0)),
        out_shape=jax.ShapeDtypeStruct((B, 2 * D), cdtype),
        scratch_shapes=[
            pltpu.VMEM((2, B, D), cdtype),
            pltpu.VMEM((4, B, H, W, Dh), cdtype),
            pltpu.VMEM((2, D, HD), cdtype),
            pltpu.VMEM((2, HD, D), cdtype),
            pltpu.VMEM((2, B, HD), cdtype),
        ],
        compiler_params=pltpu.CompilerParams(
            vmem_limit_bytes=110 * 1024 * 1024),
    )(A_x.reshape(B, D), A_k_cache, A_v_cache, A_wq, A_wo,
      B_x.reshape(B, D), B_k_cache, B_v_cache, B_wq, B_wo)
    return out.reshape(B, 1, 2 * D)
```
